```python
import os as _os
_os.environ.setdefault("JAX_PLATFORMS", "cpu")
import jax
import jax.numpy as jnp

def _softmax(x, axis=-1):
    return jax.nn.softmax(x, axis=axis)
def _gelu(x):
    return jax.nn.gelu(x, approximate=True)
def _silu(x):
    return jax.nn.silu(x)
def _sigmoid(x):
    return jax.nn.sigmoid(x)
def _layernorm(x, axis=-1, eps=1e-5):
    m = jnp.mean(x, axis=axis, keepdims=True)
    v = jnp.var(x, axis=axis, keepdims=True)
    return (x - m) / jnp.sqrt(v + eps)
def _scatter_add(tgt, idx, src, axis=0):
    return tgt.at[idx].add(src)
def _segment_sum(src, seg, n):
    return jax.ops.segment_sum(src, seg, n)
class _Rng:
    def __init__(self, key):
        self._k = key
    def _next(self):
        self._k, sub = jax.random.split(self._k)
        return sub
    def normal(self, shape):
        return jax.random.normal(self._next(), shape, dtype=jnp.bfloat16)
    def randint(self, lo, hi, shape):
        return jax.random.randint(self._next(), shape, lo, hi, dtype=jnp.int32)
    def uniform(self, shape, lo=0.0, hi=1.0):
        return jax.random.uniform(self._next(), shape, jnp.bfloat16, lo, hi)
    def permutation(self, n):
        return jax.random.permutation(self._next(), n)


kernel_name = 'interleave_layers__gqa_block_cached__dense_activation_silu__decode'

def setup_inputs():
    _rng = _Rng(jax.random.key(int.from_bytes(__import__("os").urandom(4), "little")))
    _w = (lambda a: (lambda t: t.astype(jnp.bfloat16) if jnp.issubdtype(t.dtype, jnp.floating) else t)(jnp.asarray(a)))
    def _A_setup():
        B, Sq, D = 2, 1, 512
        Hq, Hkv, Sk, Dh = 32, 8, 8192, 128
        assert Hq % Hkv == 0, (Hq, Hkv)
        return {
            "x": _w((lambda *s: _rng.normal(s) * 0.1)(B, Sq, D)),
            "k_cache": _w((lambda *s: _rng.normal(s) * 0.8)(B, Hkv, Sk, Dh)),
            "v_cache": _w((lambda *s: _rng.normal(s) * 1.6)(B, Hkv, Sk, Dh)),
            "wq": _w((lambda *s: _rng.normal(s) * 0.8)(D, Hq * Dh) * (D ** -0.5)),
            "wo": _w((lambda *s: _rng.normal(s) * 1.6)(Hq * Dh, D) * ((Hq * Dh) ** -0.5)),
        }
    _A_in = _A_setup()

    def _B_setup():
        B, S, D, F = 2, 1, 512, 1792
        return {
            "x": _w((lambda *s: _rng.normal(s) * 0.1)(B, S, D)),
            "w1": _w((lambda *s: _rng.normal(s) * 0.4)(D, F) * (D ** -0.5)),
            "w2": _w((lambda *s: _rng.normal(s) * 0.4)(F, D) * (F ** -0.5)),
        }
    _B_in = _B_setup()

    return {
        "A_x": _A_in["x"],
        "A_k_cache": _A_in["k_cache"],
        "A_v_cache": _A_in["v_cache"],
        "A_wq": _A_in["wq"],
        "A_wo": _A_in["wo"],
        "B_x": _B_in["x"],
        "B_w1": _B_in["w1"],
        "B_w2": _B_in["w2"],
    }

def reference(A_x, A_k_cache, A_v_cache, A_wq, A_wo, B_x, B_w1, B_w2):
    def _A_ref(x, k_cache, v_cache, wq, wo):
        B, Sq, D = x.shape
        Hq, Dh = 32, 128
        Hkv = k_cache.shape[1]
        rep = Hq // Hkv
        q = (lambda x, *d: x.transpose(*d))((x @ wq).reshape(B, Sq, Hq, Dh), 0, 2, 1, 3)
        k = jnp.repeat(k_cache, rep, axis=1)
        v = jnp.repeat(v_cache, rep, axis=1)
        scores = jnp.einsum("bhqd,bhkd->bhqk", q, k) * (Dh ** -0.5)
        p = _softmax(scores, axis=-1)
        o = jnp.einsum("bhqk,bhkd->bhqd", p, v)
        return (lambda x, *d: x.transpose(*d))(o, 0, 2, 1, 3).reshape(B, Sq, Hq * Dh) @ wo

    def _B_ref(x, w1, w2):
        h = jnp.einsum("bsd,df->bsf", x, w1)
        h = _silu(h)
        out = jnp.einsum("bsf,fd->bsd", h, w2)
        return out

    x = A_x
    x = x + _A_ref(_layernorm(x, axis=-1), A_k_cache, A_v_cache, A_wq, A_wo)
    x = x + _B_ref(_layernorm(x, axis=-1), B_w1, B_w2)
    x = x + _A_ref(_layernorm(x, axis=-1), A_k_cache, A_v_cache, A_wq, A_wo)
    x = x + _B_ref(_layernorm(x, axis=-1), B_w1, B_w2)
    return x
```

```python
import math

import jax
import jax.numpy as jnp
from jax import lax
import jax.experimental.pallas as pl
import jax.experimental.pallas.tpu as pltpu

B, D, HQ, HKV, SK, DH, F = 2, 512, 32, 8, 8192, 128, 1792
REP = HQ // HKV
EPS = 1e-5
C = (DH ** -0.5) * math.log2(math.e)
LAST_V_EDGES = (0, 4096, 6144, 7168, 7680, 8192)
N_LAST = len(LAST_V_EDGES) - 1

F32 = jnp.float32
BF16 = jnp.bfloat16
NT = (((1,), (1,)), ((), ()))


def _layernorm(x):
    m = jnp.mean(x, axis=-1, keepdims=True)
    d = x - m
    v = jnp.mean(d * d, axis=-1, keepdims=True)
    return d * lax.rsqrt(v + EPS)


def _kernel(x_hbm, k_hbm, v_hbm, wq_hbm, wo_hbm, w1_hbm, w2_hbm, o_ref,
            x_v, k_v, v_v, wq_v, wo_v, w1_v, w2_v, q_s, s_s, o_s,
            w_sem, k_sem, v_sem, l_sem):
    k32 = k_hbm.bitcast(jnp.uint32)
    v32 = v_hbm.bitcast(jnp.uint32)

    def k_copy(b, h):
        return pltpu.make_async_copy(k32.at[b, h], k_v.at[b, h], k_sem.at[b * HKV + h])

    def v_copy(b, h):
        return pltpu.make_async_copy(v32.at[b, h], v_v.at[b, h], v_sem.at[b * HKV + h])

    def v_piece(b, i):
        lo, hi = LAST_V_EDGES[i] // 2, LAST_V_EDGES[i + 1] // 2
        return pltpu.make_async_copy(v32.at[b, HKV - 1, pl.ds(lo, hi - lo)],
                                     v_v.at[b, HKV - 1, pl.ds(lo, hi - lo)],
                                     l_sem.at[b * N_LAST + i])

    w_copies = [pltpu.make_async_copy(s, d, w_sem.at[i]) for i, (s, d) in enumerate(
        ((x_hbm, x_v), (wq_hbm, wq_v), (wo_hbm, wo_v), (w1_hbm, w1_v), (w2_hbm, w2_v)))]

    for c in w_copies:
        c.start()
    for b in range(B):
        for h in range(HKV):
            k_copy(b, h).start()
            if h < HKV - 1:
                v_copy(b, h).start()
            else:
                for i in range(N_LAST):
                    v_piece(b, i).start()
    for c in w_copies:
        c.wait()

    row = lax.broadcasted_iota(jnp.int32, (8, DH), 0)

    def q_proj(x):
        xn = _layernorm(x).astype(BF16).astype(F32)
        q = jnp.dot(xn, wq_v[...], preferred_element_type=F32)
        for h in range(HKV):
            qh = q[:, (h * REP) * DH:(h * REP + 1) * DH]
            for j in range(1, REP):
                qh = jnp.where(row == j, q[:, (h * REP + j) * DH:(h * REP + j + 1) * DH], qh)
            q_s[h] = qh

    def load_kv(ref, b, h, lo=0, hi=SK):
        return pltpu.bitcast(ref[b, h, pl.ds(lo // 2, (hi - lo) // 2), :], BF16)

    def scores(b, h):
        return lax.dot_general(q_s[h], load_kv(k_v, b, h), NT, preferred_element_type=F32)

    def softmax_num(s):
        m = jnp.max(s, axis=1, keepdims=True)
        p = jnp.exp2((s - m) * C)
        return p, jnp.sum(p, axis=1, keepdims=True)

    def wo_part(h, o):
        acc = None
        for j in range(REP):
            w = wo_v[pl.ds(pl.multiple_of((h * REP + j) * DH, DH), DH), :]
            t = jnp.dot(jnp.where(row == j, o, 0.0), w, preferred_element_type=F32)
            acc = t if acc is None else acc + t
        return acc

    def ffn(x):
        xn = _layernorm(x).astype(BF16).astype(F32)
        a = jnp.dot(xn, w1_v[...], preferred_element_type=F32)
        a = a * jax.nn.sigmoid(a)
        return x + jnp.dot(a, w2_v[...], preferred_element_type=F32)

    def finish(x, acc):
        return ffn(x + jnp.sum(acc, axis=0, keepdims=True))

    def batch(b, carry):
        x = jnp.broadcast_to(x_v[b].astype(F32), (8, D))

        q_proj(x)

        def head1(h, acc):
            k_copy(b, h).wait()
            p, l = softmax_num(scores(b, h))
            v_copy(b, h).wait()
            o = jnp.dot(p, load_kv(v_v, b, h), preferred_element_type=F32)
            return acc + wo_part(h, o / l)

        acc = lax.fori_loop(0, HKV - 1, head1, jnp.zeros((8, D), F32))
        h = HKV - 1
        k_copy(b, h).wait()
        p, l = softmax_num(scores(b, h))
        o = None
        for i in range(N_LAST):
            lo, hi = LAST_V_EDGES[i], LAST_V_EDGES[i + 1]
            v_piece(b, i).wait()
            t = jnp.dot(p[:, lo:hi], load_kv(v_v, b, h, lo, hi), preferred_element_type=F32)
            o = t if o is None else o + t
        x = finish(x, acc + wo_part(h, o / l))

        q_proj(x)
        s_s[0] = scores(b, 0)

        def head2(h, c):
            s_s[(h + 1) % 2] = scores(b, h + 1)
            p, l = softmax_num(s_s[h % 2])
            o_s[h] = jnp.dot(p, load_kv(v_v, b, h), preferred_element_type=F32) / l
            return c

        lax.fori_loop(0, HKV - 1, head2, 0)
        acc = None
        for hh in range(HKV - 1):
            t = wo_part(hh, o_s[hh])
            acc = t if acc is None else acc + t
        p, l = softmax_num(s_s[h % 2])
        o = jnp.dot(p, load_kv(v_v, b, h), preferred_element_type=F32) / l
        x = finish(x, acc + wo_part(h, o))
        o_ref[b] = x[0:1, :].astype(o_ref.dtype)
        return carry

    lax.fori_loop(0, B, batch, 0)


@jax.jit
def pallas_interleave_layers__gqa_block_cached__dense_activation_silu__decode_kernel(
    A_x: jax.Array,
    A_k_cache: jax.Array,
    A_v_cache: jax.Array,
    A_wq: jax.Array,
    A_wo: jax.Array,
    B_x: jax.Array,
    B_w1: jax.Array,
    B_w2: jax.Array,
):
    del B_x
    hbm = pl.BlockSpec(memory_space=pltpu.HBM)
    return pl.pallas_call(
        _kernel,
        out_shape=jax.ShapeDtypeStruct(A_x.shape, A_x.dtype),
        in_specs=[hbm] * 7,
        out_specs=pl.BlockSpec(memory_space=pltpu.VMEM),
        scratch_shapes=[
            pltpu.VMEM((B, 1, D), BF16),
            pltpu.VMEM((B, HKV, SK // 2, DH), jnp.uint32),
            pltpu.VMEM((B, HKV, SK // 2, DH), jnp.uint32),
            pltpu.VMEM((D, HQ * DH), BF16),
            pltpu.VMEM((HQ * DH, D), BF16),
            pltpu.VMEM((D, F), BF16),
            pltpu.VMEM((F, D), BF16),
            pltpu.VMEM((HKV, 8, DH), F32),
            pltpu.VMEM((2, 8, SK), F32),
            pltpu.VMEM((HKV, 8, DH), F32),
            pltpu.SemaphoreType.DMA((5,)),
            pltpu.SemaphoreType.DMA((B * HKV,)),
            pltpu.SemaphoreType.DMA((B * HKV,)),
            pltpu.SemaphoreType.DMA((B * N_LAST,)),
        ],
        compiler_params=pltpu.CompilerParams(vmem_limit_bytes=100 * 1024 * 1024),
        name="gqa_ffn_two_layers",
    )(A_x, A_k_cache, A_v_cache, A_wq, A_wo, B_w1, B_w2)
```

```python
import math

import jax
import jax.numpy as jnp
from jax import lax
import jax.experimental.pallas as pl
import jax.experimental.pallas.tpu as pltpu

B, D, HQ, HKV, SK, DH, F = 2, 512, 32, 8, 8192, 128, 1792
REP = HQ // HKV
EPS = 1e-5
C = (DH ** -0.5) * math.log2(math.e)
LAST_V_EDGES = (0, 4096, 6144, 7168, 7680, 8192)
N_LAST = len(LAST_V_EDGES) - 1
AHEAD = 3

F32 = jnp.float32
BF16 = jnp.bfloat16
NT = (((1,), (1,)), ((), ()))


def _layernorm(x):
    m = jnp.mean(x, axis=-1, keepdims=True)
    d = x - m
    v = jnp.mean(d * d, axis=-1, keepdims=True)
    return d * lax.rsqrt(v + EPS)


def _kernel(x_hbm, k_hbm, v_hbm, wq_hbm, wo_hbm, w1_hbm, w2_hbm, o_ref,
            x_v, k_v, v_v, wq_v, wo_v, w1_v, w2_v, q_s, s_s, o_s,
            w_sem, k_sem, v_sem, l_sem):
    k32 = k_hbm.bitcast(jnp.uint32)
    v32 = v_hbm.bitcast(jnp.uint32)

    def k_copy(b, h):
        return pltpu.make_async_copy(k32.at[b, h], k_v.at[b, h], k_sem.at[b * HKV + h])

    def v_copy(b, h):
        return pltpu.make_async_copy(v32.at[b, h], v_v.at[b, h], v_sem.at[b * HKV + h])

    def v_piece(b, i):
        lo, hi = LAST_V_EDGES[i] // 2, LAST_V_EDGES[i + 1] // 2
        return pltpu.make_async_copy(v32.at[b, HKV - 1, pl.ds(lo, hi - lo)],
                                     v_v.at[b, HKV - 1, pl.ds(lo, hi - lo)],
                                     l_sem.at[b * N_LAST + i])

    w_copies = [pltpu.make_async_copy(s, d, w_sem.at[i]) for i, (s, d) in enumerate(
        ((x_hbm, x_v), (wq_hbm, wq_v), (wo_hbm, wo_v), (w1_hbm, w1_v), (w2_hbm, w2_v)))]

    for c in w_copies[:2]:
        c.start()
    w_copies[0].wait()
    for c in w_copies[2:] + [k_copy(0, 0)]:
        c.start()
    w_copies[1].wait()

    row = lax.broadcasted_iota(jnp.int32, (8, DH), 0)

    def q_proj(x):
        xn = _layernorm(x).astype(BF16).astype(F32)
        q = jnp.dot(xn, wq_v[...], preferred_element_type=F32)
        for h in range(HKV):
            qh = q[:, (h * REP) * DH:(h * REP + 1) * DH]
            for j in range(1, REP):
                qh = jnp.where(row == j, q[:, (h * REP + j) * DH:(h * REP + j + 1) * DH], qh)
            q_s[h] = qh

    def load_kv(ref, b, h, lo=0, hi=SK):
        return pltpu.bitcast(ref[b, h, pl.ds(lo // 2, (hi - lo) // 2), :], BF16)

    def scores(b, h):
        return lax.dot_general(q_s[h], load_kv(k_v, b, h), NT, preferred_element_type=F32)

    def softmax_num(s):
        m = jnp.max(s, axis=1, keepdims=True)
        p = jnp.exp2((s - m) * C)
        return p, jnp.sum(p, axis=1, keepdims=True)

    def wo_part(h, o):
        acc = None
        for j in range(REP):
            w = wo_v[pl.ds(pl.multiple_of((h * REP + j) * DH, DH), DH), :]
            t = jnp.dot(jnp.where(row == j, o, 0.0), w, preferred_element_type=F32)
            acc = t if acc is None else acc + t
        return acc

    def ffn(x):
        xn = _layernorm(x).astype(BF16).astype(F32)
        a = jnp.dot(xn, w1_v[...], preferred_element_type=F32)
        a = a * jax.nn.sigmoid(a)
        return x + jnp.dot(a, w2_v[...], preferred_element_type=F32)

    def finish(x, acc):
        return ffn(x + jnp.sum(acc, axis=0, keepdims=True))

    def batch(b, out):
        x = jnp.broadcast_to(x_v[...].astype(F32), (B, D))
        x = jnp.broadcast_to(jnp.where(b == 0, x[0:1], x[1:2]), (8, D))

        q_proj(x)

        @pl.when(b == 0)
        def _():
            for c in w_copies[2:]:
                c.wait()
            v_copy(0, 0).start()

        @pl.when(b == 1)
        def _():
            k_copy(1, AHEAD).start()
            v_copy(1, AHEAD).start()

        def head1(h, acc):
            fetch = jnp.logical_or(b == 0, h >= AHEAD)
            k_copy(b, h).wait()
            pl.when(fetch)(lambda: k_copy(b, h + 1).start())
            p, l = softmax_num(scores(b, h))
            v_copy(b, h).wait()
            pl.when(jnp.logical_and(fetch, h < HKV - 2))(lambda: v_copy(b, h + 1).start())
            pl.when(h == HKV - 2)(lambda: v_piece(b, 0).start())
            o = jnp.dot(p, load_kv(v_v, b, h), preferred_element_type=F32)
            return acc + wo_part(h, o / l)

        acc = lax.fori_loop(0, HKV - 1, head1, jnp.zeros((8, D), F32))
        h = HKV - 1
        k_copy(b, h).wait()
        v_piece(b, 1).start()
        p, l = softmax_num(scores(b, h))
        o = None
        for i in range(N_LAST):
            lo, hi = LAST_V_EDGES[i], LAST_V_EDGES[i + 1]
            v_piece(b, i).wait()
            if i + 2 < N_LAST:
                v_piece(b, i + 2).start()
            elif i + 2 == N_LAST:
                pl.when(b == 0)(lambda: k_copy(1, 0).start())
            else:
                @pl.when(b == 0)
                def _():
                    v_copy(1, 0).start()
                    for hh in range(1, AHEAD):
                        k_copy(1, hh).start()
                        v_copy(1, hh).start()
            t = jnp.dot(p[:, lo:hi], load_kv(v_v, b, h, lo, hi), preferred_element_type=F32)
            o = t if o is None else o + t
        x = finish(x, acc + wo_part(h, o / l))

        q_proj(x)
        s_s[0] = scores(b, 0)

        def head2(h, c):
            s_s[(h + 1) % 2] = scores(b, h + 1)
            p, l = softmax_num(s_s[h % 2])
            o_s[h] = jnp.dot(p, load_kv(v_v, b, h), preferred_element_type=F32) / l
            return c

        lax.fori_loop(0, HKV - 1, head2, 0)
        acc = None
        for hh in range(HKV - 1):
            t = wo_part(hh, o_s[hh])
            acc = t if acc is None else acc + t
        p, l = softmax_num(s_s[h % 2])
        o = jnp.dot(p, load_kv(v_v, b, h), preferred_element_type=F32) / l
        x = finish(x, acc + wo_part(h, o))
        return jnp.where(lax.broadcasted_iota(jnp.int32, (8, D), 0) == b, x, out)

    out = lax.fori_loop(0, B, batch, jnp.zeros((8, D), F32))
    o_ref[...] = out[0:B].astype(o_ref.dtype)


@jax.jit
def pallas_interleave_layers__gqa_block_cached__dense_activation_silu__decode_kernel(
    A_x: jax.Array,
    A_k_cache: jax.Array,
    A_v_cache: jax.Array,
    A_wq: jax.Array,
    A_wo: jax.Array,
    B_x: jax.Array,
    B_w1: jax.Array,
    B_w2: jax.Array,
):
    del B_x
    hbm = pl.BlockSpec(memory_space=pltpu.HBM)
    out = pl.pallas_call(
        _kernel,
        out_shape=jax.ShapeDtypeStruct((B, D), A_x.dtype),
        in_specs=[hbm] * 7,
        out_specs=pl.BlockSpec(memory_space=pltpu.VMEM),
        scratch_shapes=[
            pltpu.VMEM((B, D), BF16),
            pltpu.VMEM((B, HKV, SK // 2, DH), jnp.uint32),
            pltpu.VMEM((B, HKV, SK // 2, DH), jnp.uint32),
            pltpu.VMEM((D, HQ * DH), BF16),
            pltpu.VMEM((HQ * DH, D), BF16),
            pltpu.VMEM((D, F), BF16),
            pltpu.VMEM((F, D), BF16),
            pltpu.VMEM((HKV, 8, DH), F32),
            pltpu.VMEM((2, 8, SK), F32),
            pltpu.VMEM((HKV, 8, DH), F32),
            pltpu.SemaphoreType.DMA((5,)),
            pltpu.SemaphoreType.DMA((B * HKV,)),
            pltpu.SemaphoreType.DMA((B * HKV,)),
            pltpu.SemaphoreType.DMA((B * N_LAST,)),
        ],
        compiler_params=pltpu.CompilerParams(vmem_limit_bytes=100 * 1024 * 1024),
        name="gqa_ffn_two_layers",
    )(A_x.reshape(B, D), A_k_cache, A_v_cache, A_wq, A_wo, B_w1, B_w2)
    return out.reshape(A_x.shape)
```

```python
import functools
import math

import jax
import jax.numpy as jnp
from jax import lax
import jax.experimental.pallas as pl
import jax.experimental.pallas.tpu as pltpu

B, D, HQ, HKV, SK, DH, F = 2, 512, 32, 8, 8192, 128, 1792
REP = HQ // HKV
EPS = 1e-5
C = (DH ** -0.5) * math.log2(math.e)
LAST_V_EDGES = ((0, 8192), (0, 4096, 6144, 7680, 8192))
N_LAST = len(LAST_V_EDGES[1]) - 1
K_GROUPS = ((0, 2, 4, 6), (0, 2, 4, 5, 6, 7))
V_GROUPS = ((0, 2, 4, 6, 7), (0, 2, 4, 5, 6, 7))
DEPTH = 3
TCH = 1024
NCH = 8
LAG = 4
Q_MXU = 1
O_MXU = 2
F1V = 3
F2V = 7

F32 = jnp.float32
BF16 = jnp.bfloat16


def _layernorm(x):
    m = jnp.mean(x, axis=-1, keepdims=True)
    d = x - m
    v = jnp.mean(d * d, axis=-1, keepdims=True)
    return d * lax.rsqrt(v + EPS)


def _kernel(x_hbm, k_hbm, v_hbm, wq_hbm, wo_hbm, w1_hbm, w2_hbm, o_ref,
            x_v, k_v, v_v, wq_v, wo_v, w1_v, w2_v, kt_v, q_s, p_s, l_s, wq_f, wo_f, w1_f, w2_f,
            sem):
    k32 = k_hbm.bitcast(jnp.uint32)
    v32 = v_hbm.bitcast(jnp.uint32)

    order = [("x", x_hbm, x_v), ("wq", wq_hbm.bitcast(jnp.uint32), wq_v)]
    for b in range(B):
        for h in range(-1, HKV):
            for tag, src, dst, groups, g in (("k", k32, k_v, K_GROUPS[b], h + 1), ("v", v32, v_v, V_GROUPS[b], h)):
                if g not in groups:
                    continue
                n = (groups + (HKV,))[groups.index(g) + 1] - g
                if tag == "v" and g == HKV - 1:
                    e = LAST_V_EDGES[b]
                    for i in range(len(e) - 1):
                        rows = pl.ds(e[i] // 2, (e[i + 1] - e[i]) // 2)
                        order.append((("p", b, i), src.at[b, g, rows], dst.at[b, g, rows]))
                else:
                    order.append(((tag, b, g), src.at[b, pl.ds(g, n)], dst.at[b, pl.ds(g, n)]))
                if (tag, b, g) == ("v", 0, 0):
                    order.append(("wo", wo_hbm.bitcast(jnp.uint32), wo_v))
        if b == 0:
            order += [("w1", w1_hbm.bitcast(jnp.uint32), w1_v), ("w2", w2_hbm.bitcast(jnp.uint32), w2_v)]
    copies = [pltpu.make_async_copy(s, d, sem.at[i % DEPTH]) for i, (_, s, d) in enumerate(order)]
    index = {key: i for i, (key, _, _) in enumerate(order)}

    def arrive(key):
        i = index[key]
        copies[i].wait()
        if i + DEPTH < len(copies):
            copies[i + DEPTH].start()

    def arrive_head(tag, b, h):
        for bb, groups in enumerate(K_GROUPS if tag == "k" else V_GROUPS):
            for g in groups:
                if (tag, bb, g) in index and not (isinstance(h, int) and h != g):
                    pl.when(jnp.logical_and(b == bb, h == g))(lambda: arrive((tag, bb, g)))

    for c in copies[:DEPTH]:
        c.start()
    arrive("x")
    arrive("wq")

    row = lax.broadcasted_iota(jnp.int32, (8, DH), 0)

    def q_proj(x):
        xn = _layernorm(x).astype(BF16).astype(F32)
        q = jnp.dot(xn, pltpu.bitcast(wq_v[...], BF16), preferred_element_type=F32)
        return [pick_rows(q[:, h * REP * DH:(h + 1) * REP * DH]) for h in range(HKV)]

    def pick_rows(q):
        qh = jnp.broadcast_to(q[:, 0:DH], (8, DH))
        for j in range(1, REP):
            qh = jnp.where(row == j, q[:, j * DH:(j + 1) * DH], qh)
        return qh

    def lane_bcast(r):
        t = jnp.broadcast_to(r, (DH, DH)).astype(BF16).T
        return pltpu.bitcast(t, jnp.uint32)

    def unpack(w):
        lo = pltpu.bitcast(w << 16, F32)
        hi = pltpu.bitcast(w & jnp.uint32(0xFFFF0000), F32)
        return lo, hi

    def widen(dst, src, r0, c0):
        cols = dst.shape[1]

        def body(i, carry):
            lo, hi = unpack(src[pl.ds(pl.multiple_of(r0 + i * 8, 8), 8), c0:c0 + cols])
            dst[pl.ds(pl.multiple_of(i * 16, 16), 8), :] = lo
            dst[pl.ds(pl.multiple_of(i * 16 + 8, 8), 8), :] = hi
            return carry

        lax.fori_loop(0, dst.shape[0] // 16, body, 0)

    def bcast_rows(r):
        t = lane_bcast(r)
        return [v for i in range(0, DH // 2, 8) for v in unpack(t[i:i + 8])]

    def vpu_rows(w_ref, r0, c0, xs, accs):
        for i, xv in enumerate(xs):
            for c in range(len(accs)):
                t = w_ref[r0 + i * 8:r0 + i * 8 + 8, c0 + c * DH:c0 + (c + 1) * DH] * xv
                accs[c] = t if accs[c] is None else accs[c] + t

    def load_kv(ref, b, h, lo=0, hi=SK):
        return pltpu.bitcast(ref[b, h, pl.ds(lo // 2, (hi - lo) // 2), :], BF16)

    def transpose_k(b, h):
        for c in range(0, SK, TCH):
            kt_v[h, :, c:c + TCH] = pltpu.bitcast(load_kv(k_v, b, h, c, c + TCH).T, jnp.uint32)

    def scores(q, h):
        return jnp.dot(q, pltpu.bitcast(kt_v[h], BF16), preferred_element_type=F32)

    def softmax_num(s):
        m = jnp.max(s, axis=1, keepdims=True)
        p = jnp.exp2((s - m) * C)
        return p, jnp.sum(p, axis=1, keepdims=True)

    def wo_part(h, o):
        acc = None
        for j in range(REP):
            start = (h * REP + j) * (DH // 2)
            if not isinstance(h, int):
                start = pl.multiple_of(start, DH // 2)
            w = pltpu.bitcast(wo_v[pl.ds(start, DH // 2), :], BF16)
            t = jnp.dot(jnp.where(row == j, o, 0.0), w, preferred_element_type=F32)
            acc = t if acc is None else acc + t
        return acc

    def ffn(x):
        xn = _layernorm(x).astype(BF16).astype(F32)
        nb = F // DH
        silu = lambda a: a * jax.nn.sigmoid(a)

        def up(lo, hi):
            w = pltpu.bitcast(w1_v[:, lo * DH:hi * DH], BF16)
            return silu(jnp.dot(xn, w, preferred_element_type=F32))

        def down(a, lo, hi):
            w = pltpu.bitcast(w2_v[lo * 64:hi * 64, :], BF16)
            return jnp.dot(a, w, preferred_element_type=F32)

        a0 = up(0, F2V)
        a1 = up(F2V, nb - F1V)
        accs = [None] * F1V
        for c in range(D // DH):
            vpu_rows(w1_f, c * DH, 0, bcast_rows(xn[0:1, c * DH:(c + 1) * DH]), accs)
        a2 = jnp.concatenate([jnp.sum(a, axis=0, keepdims=True) for a in accs], axis=1)
        a2 = jnp.broadcast_to(silu(a2), (8, F1V * DH))
        y = x + down(a1, F2V, nb - F1V)
        accs = [None] * (D // DH)
        for j in range(F2V):
            vpu_rows(w2_f, j * DH, 0, bcast_rows(a0[0:1, j * DH:(j + 1) * DH]), accs)
        y = y + jnp.sum(jnp.concatenate(accs, axis=1), axis=0, keepdims=True)
        y = y + down(a2, nb - F1V, nb)
        return y

    def finish(x, acc):
        return ffn(x + jnp.sum(acc, axis=0, keepdims=True))

    def batch(b, out):
        x = x_v[...].astype(F32)
        x = jnp.broadcast_to(jnp.where(b == 0, x[0:1], x[1:2]), (8, D))

        for h, q in enumerate(q_proj(x)):
            q_s[h] = q

        def probs(h):
            arrive_head("k", b, h)
            transpose_k(b, h)
            p, l = softmax_num(scores(q_s[h], h))
            p_s[h % 2] = p
            l_s[h % 2] = jnp.broadcast_to(l, (8, DH))

        probs(0)

        def head1(h, acc):
            probs(h + 1)
            arrive_head("v", b, h)

            @pl.when(jnp.logical_and(b == 0, h == 0))
            def _():
                widen(wq_f, wq_v, 0, Q_MXU * REP * DH)
                arrive("wo")
                widen(wo_f, wo_v, 0, 0)

            o = jnp.dot(p_s[h % 2], load_kv(v_v, b, h), preferred_element_type=F32)
            return acc + wo_part(h, o / l_s[h % 2])

        acc = lax.fori_loop(0, HKV - 1, head1, jnp.zeros((8, D), F32))

        h = HKV - 1
        p, l = p_s.at[h % 2], l_s[h % 2]
        o = None
        for i in range(N_LAST):
            lo, hi = LAST_V_EDGES[1][i], LAST_V_EDGES[1][i + 1]
            for bb in range(B):
                if ("p", bb, i) in index:
                    pl.when(b == bb)(lambda: arrive(("p", bb, i)))
            if i == 0:
                @pl.when(b == 0)
                def _():
                    arrive("w1")
                    widen(w1_f, w1_v, 0, F - F1V * DH)
                    arrive("w2")
                    widen(w2_f, w2_v, 0, 0)
            t = jnp.dot(p[:, lo:hi], load_kv(v_v, b, h, lo, hi), preferred_element_type=F32)
            o = t if o is None else o + t
        x = finish(x, acc + wo_part(h, o / l))

        xn = _layernorm(x).astype(BF16).astype(F32)
        q = {}
        o_all = {}
        for h in range(Q_MXU):
            w = pltpu.bitcast(wq_v[:, h * REP * DH:(h + 1) * REP * DH], BF16)
            q[h] = pick_rows(jnp.dot(xn, w, preferred_element_type=F32))
        xs = [bcast_rows(xn[0:1, c * DH:(c + 1) * DH]) for c in range(D // DH)]
        acc = [None] * (D // DH)

        def q_tasks(h):
            accs = [None] * REP

            def part(i):
                vpu_rows(wq_f, i * DH, (h - Q_MXU) * REP * DH, xs[i], accs)
                if i == 3:
                    q[h] = pick_rows(jnp.concatenate([jnp.sum(a, axis=0, keepdims=True) for a in accs], axis=1))
                return accs
            return [functools.partial(part, i) for i in range(4)]

        def o_tasks(h, o):
            def part(j):
                vpu_rows(wo_f, (h * REP + j) * DH, 0, bcast_rows(o[j:j + 1, :]), acc)
                return acc
            return [functools.partial(part, j) for j in range(REP)]

        ch = SK // NCH

        always = row >= (b >> 1)
        pinned = {}

        def pin(slot, tasks, step=1):
            for i, t in enumerate(tasks):
                pinned.setdefault(slot + i * step, []).append(t)

        def run(slot, lhs):
            for t in pinned.pop(slot, []):
                for a in t():
                    lhs = None if lhs is None else jnp.where(always, lhs, a)
            return lhs

        def qk(h):
            s = []
            for c in range(NCH):
                kt = pltpu.bitcast(kt_v[h, :, c * ch:(c + 1) * ch], BF16)
                qc = run(max(2 * h - 1, 0) * NCH + c, None if c == 0 and h == 1 else q[h])
                qc = q[h] if qc is None else qc
                s.append(jnp.dot(qc, kt, preferred_element_type=F32))
            return s

        def pv(h, s):
            m = s[0]
            for t in s[1:]:
                m = jnp.maximum(m, t)
            m = jnp.broadcast_to(jnp.max(m, axis=1, keepdims=True), (8, DH))
            o = l = None
            ts = []
            for c in range(NCH):
                mc = run((2 * h + 2) * NCH + c, m)
                if c >= LAG:
                    mc = jnp.where(always, mc, ts[c - LAG])
                p = jnp.exp2((s[c] - jnp.tile(mc, (1, ch // DH))) * C)
                t = jnp.dot(p, load_kv(v_v, b, h, c * ch, (c + 1) * ch), preferred_element_type=F32)
                ts.append(t)
                o = t if o is None else o + t
                l = p if l is None else l + p
            return o / jnp.sum(l, axis=1, keepdims=True)

        step = NCH // 4
        for h in range(Q_MXU, HKV):
            pin(max((2 * h - 3) * NCH, 0) + step, q_tasks(h), step)
        s = qk(0)
        acc_m = None
        for h in range(HKV):
            s_next = qk(h + 1) if h + 1 < HKV else None
            if h == HKV - 1:
                for hh in range(HKV - O_MXU, HKV - 1):
                    t = wo_part(hh, o_all[hh])
                    acc_m = t if acc_m is None else acc_m + t
            o_prev = o_all[h] = pv(h, s)
            if h < HKV - O_MXU:
                pin((2 * h + 4) * NCH + step - (NCH if h == HKV - 2 else 0), o_tasks(h, o_prev), step)
            s = s_next
        for ts in list(pinned.values()):
            for t in ts:
                t()
        t = wo_part(HKV - 1, o_prev)
        acc_m = t if acc_m is None else acc_m + t
        acc_m = acc_m + jnp.concatenate(acc, axis=1)
        x = finish(x, acc_m)
        return jnp.where(lax.broadcasted_iota(jnp.int32, (8, D), 0) == b, x, out)

    out = lax.fori_loop(0, B, batch, jnp.zeros((8, D), F32))
    o_ref[...] = out[0:B].astype(o_ref.dtype)


@jax.jit
def pallas_interleave_layers__gqa_block_cached__dense_activation_silu__decode_kernel(
    A_x: jax.Array,
    A_k_cache: jax.Array,
    A_v_cache: jax.Array,
    A_wq: jax.Array,
    A_wo: jax.Array,
    B_x: jax.Array,
    B_w1: jax.Array,
    B_w2: jax.Array,
):
    del B_x
    hbm = pl.BlockSpec(memory_space=pltpu.HBM)
    out = pl.pallas_call(
        _kernel,
        out_shape=jax.ShapeDtypeStruct((B, D), A_x.dtype),
        in_specs=[hbm] * 7,
        out_specs=pl.BlockSpec(memory_space=pltpu.VMEM),
        scratch_shapes=[
            pltpu.VMEM((B, D), BF16),
            pltpu.VMEM((B, HKV, SK // 2, DH), jnp.uint32),
            pltpu.VMEM((B, HKV, SK // 2, DH), jnp.uint32),
            pltpu.VMEM((D // 2, HQ * DH), jnp.uint32),
            pltpu.VMEM((HQ * DH // 2, D), jnp.uint32),
            pltpu.VMEM((D // 2, F), jnp.uint32),
            pltpu.VMEM((F // 2, D), jnp.uint32),
            pltpu.VMEM((HKV, DH // 2, SK), jnp.uint32),
            pltpu.VMEM((HKV, 8, DH), F32),
            pltpu.VMEM((2, 8, SK), F32),
            pltpu.VMEM((2, 8, DH), F32),
            pltpu.VMEM((D, (HKV - Q_MXU) * REP * DH), F32),
            pltpu.VMEM(((HKV - O_MXU) * REP * DH, D), F32),
            pltpu.VMEM((D, F1V * DH), F32),
            pltpu.VMEM((F2V * DH, D), F32),
            pltpu.SemaphoreType.DMA((DEPTH,)),
        ],
        compiler_params=pltpu.CompilerParams(
            vmem_limit_bytes=120 * 1024 * 1024,
            flags={"XLA_TPU_FORCE_LP_LLO_SCHEDULER": True},
        ),
        name="gqa_ffn_two_layers",
    )(A_x.reshape(B, D), A_k_cache, A_v_cache, A_wq, A_wo, B_w1, B_w2)
    return out.reshape(A_x.shape)
```

```python
import functools
import math

import jax
import jax.numpy as jnp
from jax import lax
import jax.experimental.pallas as pl
import jax.experimental.pallas.tpu as pltpu

B, D, HQ, HKV, SK, DH, F = 2, 512, 32, 8, 8192, 128, 1792
REP = HQ // HKV
EPS = 1e-5
C = (DH ** -0.5) * math.log2(math.e)
LAST_V_EDGES = ((0, 8192), (0, 4096, 6144, 7680, 8192))
N_LAST = len(LAST_V_EDGES[1]) - 1
K_GROUPS = ((0, 2, 4, 6), (0, 2, 4, 5, 6, 7))
V_GROUPS = ((0, 2, 4, 6, 7), (0, 2, 4, 5, 6, 7))
DEPTH = 3
TCH = 1024
NCH = 8
LAG = 4
Q_MXU = 1
O_MXU = 2
F1V = 3
F2V = 7

F32 = jnp.float32
BF16 = jnp.bfloat16


def _layernorm(x):
    m = jnp.mean(x, axis=-1, keepdims=True)
    d = x - m
    v = jnp.mean(d * d, axis=-1, keepdims=True)
    return d * lax.rsqrt(v + EPS)


def _kernel(x_hbm, k_hbm, v_hbm, wq_hbm, wo_hbm, w1_hbm, w2_hbm, o_ref,
            x_v, k_v, v_v, wq_v, wo_v, w1_v, w2_v, kt_v, q_s, p_s, l_s, vt_v, wq_f, wo_f, w1_f, w2_f,
            sem):
    order = [("x", x_hbm, x_v), ("wq", wq_hbm, wq_v)]
    for b in range(B):
        for h in range(-1, HKV):
            for tag, src, dst, groups, g in (("k", k_hbm, k_v, K_GROUPS[b], h + 1), ("v", v_hbm, v_v, V_GROUPS[b], h)):
                if g not in groups:
                    continue
                n = (groups + (HKV,))[groups.index(g) + 1] - g
                if tag == "v" and g == HKV - 1:
                    e = LAST_V_EDGES[b]
                    for i in range(len(e) - 1):
                        rows = pl.ds(e[i], e[i + 1] - e[i])
                        order.append((("p", b, i), src.at[b, g, rows], dst.at[b, g, rows]))
                else:
                    order.append(((tag, b, g), src.at[b, pl.ds(g, n)], dst.at[b, pl.ds(g, n)]))
                if (tag, b, g) == ("v", 0, 0):
                    order.append(("wo", wo_hbm, wo_v))
        if b == 0:
            order += [("w1", w1_hbm, w1_v), ("w2", w2_hbm, w2_v)]
    copies = [pltpu.make_async_copy(s, d, sem.at[i % DEPTH]) for i, (_, s, d) in enumerate(order)]
    index = {key: i for i, (key, _, _) in enumerate(order)}

    def arrive(key):
        i = index[key]
        copies[i].wait()
        if i + DEPTH < len(copies):
            copies[i + DEPTH].start()

    def arrive_head(tag, b, h):
        for bb, groups in enumerate(K_GROUPS if tag == "k" else V_GROUPS):
            for g in groups:
                if (tag, bb, g) in index and not (isinstance(h, int) and h != g):
                    pl.when(jnp.logical_and(b == bb, h == g))(lambda: arrive((tag, bb, g)))

    for c in copies[:DEPTH]:
        c.start()
    arrive("x")
    arrive("wq")

    row = lax.broadcasted_iota(jnp.int32, (8, DH), 0)

    def q_proj(x):
        xn = _layernorm(x).astype(BF16).astype(F32)
        q = jnp.dot(xn, wq_v[...], preferred_element_type=F32)
        return [pick_rows(q[:, h * REP * DH:(h + 1) * REP * DH]) for h in range(HKV)]

    def pick_rows(q):
        qh = jnp.broadcast_to(q[:, 0:DH], (8, DH))
        for j in range(1, REP):
            qh = jnp.where(row == j, q[:, j * DH:(j + 1) * DH], qh)
        return qh

    def lane_bcast(r):
        t = jnp.broadcast_to(r, (DH, DH)).astype(BF16).T
        return pltpu.bitcast(t, jnp.uint32)

    def unpack(w):
        lo = pltpu.bitcast(w << 16, F32)
        hi = pltpu.bitcast(w & jnp.uint32(0xFFFF0000), F32)
        return lo, hi

    def widen(dst, src, r0, c0):
        cols = dst.shape[1]

        def body(i, carry):
            lo, hi = unpack(pltpu.bitcast(src[pl.ds(pl.multiple_of(r0 + i * 16, 16), 16), c0:c0 + cols], jnp.uint32))
            dst[pl.ds(pl.multiple_of(i * 16, 16), 8), :] = lo
            dst[pl.ds(pl.multiple_of(i * 16 + 8, 8), 8), :] = hi
            return carry

        lax.fori_loop(0, dst.shape[0] // 16, body, 0)

    def bcast_rows(r):
        t = lane_bcast(r)
        return [v for i in range(0, DH // 2, 8) for v in unpack(t[i:i + 8])]

    def vpu_rows(w_ref, r0, c0, xs, accs):
        for i, xv in enumerate(xs):
            for c in range(len(accs)):
                t = w_ref[r0 + i * 8:r0 + i * 8 + 8, c0 + c * DH:c0 + (c + 1) * DH] * xv
                accs[c] = t if accs[c] is None else accs[c] + t

    def load_kv(ref, b, h, lo=0, hi=SK):
        return ref[b, h, pl.ds(lo, hi - lo), :]

    def transpose_k(b, h):
        for c in range(0, SK, TCH):
            kt_v[h, :, c:c + TCH] = pltpu.bitcast(load_kv(k_v, b, h, c, c + TCH).T, jnp.uint32)

    def scores(q, h):
        return jnp.dot(q, pltpu.bitcast(kt_v[h], BF16), preferred_element_type=F32)

    def softmax_num(s):
        m = jnp.max(s, axis=1, keepdims=True)
        p = jnp.exp2((s - m) * C)
        return p, jnp.sum(p, axis=1, keepdims=True)

    def wo_part(h, o):
        acc = None
        for j in range(REP):
            start = (h * REP + j) * DH
            if not isinstance(h, int):
                start = pl.multiple_of(start, DH)
            w = wo_v[pl.ds(start, DH), :]
            t = jnp.dot(jnp.where(row == j, o, 0.0), w, preferred_element_type=F32)
            acc = t if acc is None else acc + t
        return acc

    def ffn(x):
        xn = _layernorm(x).astype(BF16).astype(F32)
        nb = F // DH
        silu = lambda a: a * jax.nn.sigmoid(a)

        def up(lo, hi):
            w = w1_v[:, lo * DH:hi * DH]
            return silu(jnp.dot(xn, w, preferred_element_type=F32))

        def down(a, lo, hi):
            w = w2_v[lo * DH:hi * DH, :]
            return jnp.dot(a, w, preferred_element_type=F32)

        a0 = up(0, F2V)
        a1 = up(F2V, nb - F1V)
        accs = [None] * F1V
        for c in range(D // DH):
            vpu_rows(w1_f, c * DH, 0, bcast_rows(xn[0:1, c * DH:(c + 1) * DH]), accs)
        a2 = jnp.concatenate([jnp.sum(a, axis=0, keepdims=True) for a in accs], axis=1)
        a2 = jnp.broadcast_to(silu(a2), (8, F1V * DH))
        y = x + down(a1, F2V, nb - F1V)
        accs = [None] * (D // DH)
        for j in range(F2V):
            vpu_rows(w2_f, j * DH, 0, bcast_rows(a0[0:1, j * DH:(j + 1) * DH]), accs)
        y = y + jnp.sum(jnp.concatenate(accs, axis=1), axis=0, keepdims=True)
        y = y + down(a2, nb - F1V, nb)
        return y

    def finish(x, acc):
        return ffn(x + jnp.sum(acc, axis=0, keepdims=True))

    def batch(b, out):
        x = x_v[...].astype(F32)
        x = jnp.broadcast_to(jnp.where(b == 0, x[0:1], x[1:2]), (8, D))

        for h, q in enumerate(q_proj(x)):
            q_s[h] = q

        def probs(h):
            arrive_head("k", b, h)
            transpose_k(b, h)
            p, l = softmax_num(scores(q_s[h], h))
            p_s[h % 2] = p
            l_s[h % 2] = jnp.broadcast_to(l, (8, DH))

        probs(0)

        def head1(h, acc):
            probs(h + 1)
            arrive_head("v", b, h)

            @pl.when(jnp.logical_and(b == 0, h == 0))
            def _():
                widen(wq_f, wq_v, 0, Q_MXU * REP * DH)
                arrive("wo")
                widen(wo_f, wo_v, 0, 0)

            v = load_kv(v_v, b, h)
            vt_v[h] = pltpu.bitcast(v, jnp.uint32)
            o = jnp.dot(p_s[h % 2], v, preferred_element_type=F32)
            return acc + wo_part(h, o / l_s[h % 2])

        acc = lax.fori_loop(0, HKV - 1, head1, jnp.zeros((8, D), F32))

        h = HKV - 1
        p, l = p_s.at[h % 2], l_s[h % 2]
        o = None
        for i in range(N_LAST):
            lo, hi = LAST_V_EDGES[1][i], LAST_V_EDGES[1][i + 1]
            for bb in range(B):
                if ("p", bb, i) in index:
                    pl.when(b == bb)(lambda: arrive(("p", bb, i)))
            if i == 0:
                @pl.when(b == 0)
                def _():
                    arrive("w1")
                    widen(w1_f, w1_v, 0, F - F1V * DH)
                    arrive("w2")
                    widen(w2_f, w2_v, 0, 0)
            t = jnp.dot(p[:, lo:hi], load_kv(v_v, b, h, lo, hi), preferred_element_type=F32)
            o = t if o is None else o + t
        x = finish(x, acc + wo_part(h, o / l))

        xn = _layernorm(x).astype(BF16).astype(F32)
        q = {}
        o_all = {}
        for h in range(Q_MXU):
            w = wq_v[:, h * REP * DH:(h + 1) * REP * DH]
            q[h] = pick_rows(jnp.dot(xn, w, preferred_element_type=F32))
        xs = [bcast_rows(xn[0:1, c * DH:(c + 1) * DH]) for c in range(D // DH)]
        acc = [None] * (D // DH)

        def q_tasks(h):
            accs = [None] * REP

            def part(i):
                vpu_rows(wq_f, i * DH, (h - Q_MXU) * REP * DH, xs[i], accs)
                if i == 3:
                    q[h] = pick_rows(jnp.concatenate([jnp.sum(a, axis=0, keepdims=True) for a in accs], axis=1))
                return accs
            return [functools.partial(part, i) for i in range(4)]

        def o_tasks(h, o):
            def part(j):
                vpu_rows(wo_f, (h * REP + j) * DH, 0, bcast_rows(o[j:j + 1, :]), acc)
                return acc
            return [functools.partial(part, j) for j in range(REP)]

        ch = SK // NCH

        always = row >= (b >> 1)
        pinned = {}

        def pin(slot, tasks, step=1):
            for i, t in enumerate(tasks):
                pinned.setdefault(slot + i * step, []).append(t)

        def run(slot, lhs):
            for t in pinned.pop(slot, []):
                for a in t():
                    lhs = None if lhs is None else jnp.where(always, lhs, a)
            return lhs

        def qk(h):
            s = []
            for c in range(NCH):
                kt = pltpu.bitcast(kt_v[h, :, c * ch:(c + 1) * ch], BF16)
                qc = run(max(2 * h - 1, 0) * NCH + c, None if c == 0 and h == 1 else q[h])
                qc = q[h] if qc is None else qc
                s.append(jnp.dot(qc, kt, preferred_element_type=F32))
            return s

        def pv(h, s):
            m = s[0]
            for t in s[1:]:
                m = jnp.maximum(m, t)
            m = jnp.broadcast_to(jnp.max(m, axis=1, keepdims=True), (8, DH))
            o = l = None
            ts = []
            for c in range(NCH):
                mc = run((2 * h + 2) * NCH + c, m)
                if c >= LAG:
                    mc = jnp.where(always, mc, ts[c - LAG])
                p = jnp.exp2((s[c] - jnp.tile(mc, (1, ch // DH))) * C)
                v = (pltpu.bitcast(vt_v[h, c * ch // 2:(c + 1) * ch // 2, :], BF16) if h < HKV - 1
                     else load_kv(v_v, b, h, c * ch, (c + 1) * ch))
                t = jnp.dot(p, v, preferred_element_type=F32)
                ts.append(t)
                o = t if o is None else o + t
                l = p if l is None else l + p
            return o / jnp.sum(l, axis=1, keepdims=True)

        step = NCH // 4
        for h in range(Q_MXU, HKV):
            pin(max((2 * h - 3) * NCH, 0) + step, q_tasks(h), step)
        s = qk(0)
        acc_m = None
        for h in range(HKV):
            s_next = qk(h + 1) if h + 1 < HKV else None
            if h == HKV - 1:
                for hh in range(HKV - O_MXU, HKV - 1):
                    t = wo_part(hh, o_all[hh])
                    acc_m = t if acc_m is None else acc_m + t
            o_prev = o_all[h] = pv(h, s)
            if h < HKV - O_MXU:
                pin((2 * h + 4) * NCH + step - (NCH if h == HKV - 2 else 0), o_tasks(h, o_prev), step)
            s = s_next
        for ts in list(pinned.values()):
            for t in ts:
                t()
        t = wo_part(HKV - 1, o_prev)
        acc_m = t if acc_m is None else acc_m + t
        acc_m = acc_m + jnp.concatenate(acc, axis=1)
        x = finish(x, acc_m)
        return jnp.where(lax.broadcasted_iota(jnp.int32, (8, D), 0) == b, x, out)

    out = lax.fori_loop(0, B, batch, jnp.zeros((8, D), F32))
    o_ref[...] = out[0:B].astype(o_ref.dtype)


@jax.jit
def pallas_interleave_layers__gqa_block_cached__dense_activation_silu__decode_kernel(
    A_x: jax.Array,
    A_k_cache: jax.Array,
    A_v_cache: jax.Array,
    A_wq: jax.Array,
    A_wo: jax.Array,
    B_x: jax.Array,
    B_w1: jax.Array,
    B_w2: jax.Array,
):
    del B_x
    hbm = pl.BlockSpec(memory_space=pltpu.HBM)
    out = pl.pallas_call(
        _kernel,
        out_shape=jax.ShapeDtypeStruct((B, D), A_x.dtype),
        in_specs=[hbm] * 7,
        out_specs=pl.BlockSpec(memory_space=pltpu.VMEM),
        scratch_shapes=[
            pltpu.VMEM((B, D), BF16),
            pltpu.VMEM((B, HKV, SK, DH), BF16),
            pltpu.VMEM((B, HKV, SK, DH), BF16),
            pltpu.VMEM((D, HQ * DH), BF16),
            pltpu.VMEM((HQ * DH, D), BF16),
            pltpu.VMEM((D, F), BF16),
            pltpu.VMEM((F, D), BF16),
            pltpu.VMEM((HKV, DH // 2, SK), jnp.uint32),
            pltpu.VMEM((HKV, 8, DH), F32),
            pltpu.VMEM((2, 8, SK), F32),
            pltpu.VMEM((2, 8, DH), F32),
            pltpu.VMEM((HKV - 1, SK // 2, DH), jnp.uint32),
            pltpu.VMEM((D, (HKV - Q_MXU) * REP * DH), F32),
            pltpu.VMEM(((HKV - O_MXU) * REP * DH, D), F32),
            pltpu.VMEM((D, F1V * DH), F32),
            pltpu.VMEM((F2V * DH, D), F32),
            pltpu.SemaphoreType.DMA((DEPTH,)),
        ],
        compiler_params=pltpu.CompilerParams(
            vmem_limit_bytes=126 * 1024 * 1024,
            flags={"XLA_TPU_FORCE_LP_LLO_SCHEDULER": True},
        ),
        name="gqa_ffn_two_layers",
    )(A_x.reshape(B, D), A_k_cache, A_v_cache, A_wq, A_wo, B_w1, B_w2)
    return out.reshape(A_x.shape)
```
